```python
import os as _os
_os.environ.setdefault("JAX_PLATFORMS", "cpu")
import jax
import jax.numpy as jnp

def _softmax(x, axis=-1):
    return jax.nn.softmax(x, axis=axis)
def _gelu(x):
    return jax.nn.gelu(x, approximate=True)
def _silu(x):
    return jax.nn.silu(x)
def _sigmoid(x):
    return jax.nn.sigmoid(x)
def _layernorm(x, axis=-1, eps=1e-5):
    m = jnp.mean(x, axis=axis, keepdims=True)
    v = jnp.var(x, axis=axis, keepdims=True)
    return (x - m) / jnp.sqrt(v + eps)
def _scatter_add(tgt, idx, src, axis=0):
    return tgt.at[idx].add(src)
def _segment_sum(src, seg, n):
    return jax.ops.segment_sum(src, seg, n)
class _Rng:
    def __init__(self, key):
        self._k = key
    def _next(self):
        self._k, sub = jax.random.split(self._k)
        return sub
    def normal(self, shape):
        return jax.random.normal(self._next(), shape, dtype=jnp.bfloat16)
    def randint(self, lo, hi, shape):
        return jax.random.randint(self._next(), shape, lo, hi, dtype=jnp.int32)
    def uniform(self, shape, lo=0.0, hi=1.0):
        return jax.random.uniform(self._next(), shape, jnp.bfloat16, lo, hi)
    def permutation(self, n):
        return jax.random.permutation(self._next(), n)


kernel_name = 'standalone__seq2seq_rnn_t_joint__speech'

def setup_inputs():
    _rng = _Rng(jax.random.key(int.from_bytes(__import__("os").urandom(4), "little")))
    _w = (lambda a: (lambda t: t.astype(jnp.bfloat16) if jnp.issubdtype(t.dtype, jnp.floating) else t)(jnp.asarray(a)))
    B, T, D, K = 2, 1000, 512, 31
    U = 8
    sc = (1.0 / (K * D)) ** 0.5
    sd = (1.0 / D) ** 0.5
    return {
        "x": _w((lambda *s: _rng.normal(s) * 0.4)(B, T, D) * 0.5),
        "w1": _w((lambda *s: _rng.normal(s) * 1.6)(K, D, D) * sc),
        "w2": _w((lambda *s: _rng.normal(s) * 1.6)(K, D, D) * sc),
        "g": _w((lambda *s: _rng.normal(s) * 1.6)(B, U, D) * 0.5),
        "w_f": _w((lambda *s: _rng.normal(s) * 1.6)(D, D) * sd),
        "w_g": _w((lambda *s: _rng.normal(s) * 1.6)(D, D) * sd),
        "w_o": _w((lambda *s: _rng.normal(s) * 1.6)(D, D) * sd),
    }

def reference(x, w1, w2, g, w_f, w_g, w_o):
    B, T, D = x.shape
    K = w1.shape[0]
    pad = K // 2
    xp = jnp.pad(x, ((0,0),(pad,pad),(0,0)))
    h = jnp.zeros_like(x)
    for i in range(K):
        h = h + jnp.einsum("btc,cd->btd", xp[:, i:i+T, :], w1[i])
    h = _gelu(h)[:, ::2, :]
    T1 = h.shape[1]
    hp = jnp.pad(h, ((0,0),(pad,pad),(0,0)))
    f = jnp.zeros_like(h)
    for i in range(K):
        f = f + jnp.einsum("btc,cd->btd", hp[:, i:i+T1, :], w2[i])
    f = _gelu(f)[:, ::2, :]
    fe = jnp.einsum("btd,de->bte", f, w_f)
    ge = jnp.einsum("bud,de->bue", g, w_g)
    j = jnp.tanh(fe[:, :, None, :] + ge[:, None, :, :])
    return jnp.einsum("btud,dv->btuv", j, w_o)
```

```python
import numpy as np
import jax
import jax.numpy as jnp
import jax.experimental.pallas as pl
import jax.experimental.pallas.tpu as pltpu

F32 = jnp.float32
BF16 = jnp.bfloat16

L1 = 3
L2 = 2


def _w_terms(L):
    G = np.array([[1, 0], [1, 1], [0, 1]])
    M = np.eye(1, dtype=int)
    for _ in range(L):
        M = np.kron(G, M)
    return [[int(t) for t in np.nonzero(r)[0]] for r in M]


def _x_tree(xs):
    if len(xs) == 1:
        return list(xs)
    h = (len(xs) + 1) // 4
    n = 2 * h - 1
    x0, x1, x2 = xs[0:n], xs[h:h + n], xs[2 * h:2 * h + n]
    return (_x_tree([a - b for a, b in zip(x0, x1)]) + _x_tree(list(x1))
            + _x_tree([a - b for a, b in zip(x2, x1)]))


def _y_tree(ys):
    if len(ys) == 1:
        return list(ys)
    n = len(ys) // 3
    a, b, c = _y_tree(ys[:n]), _y_tree(ys[n:2 * n]), _y_tree(ys[2 * n:])
    return [u + v for u, v in zip(a, b)] + [u + v for u, v in zip(b, c)]


def _gelu(x):
    c = float(np.sqrt(2.0 / np.pi))
    return 0.5 * x * (1.0 + jnp.tanh(c * (x + 0.044715 * (x * x * x))))


@jax.jit
def pallas_standalone__seq2seq_rnn_t_joint__speech_kernel(
    x: jax.Array,
    w1: jax.Array,
    w2: jax.Array,
    g: jax.Array,
    w_f: jax.Array,
    w_g: jax.Array,
    w_o: jax.Array,
):
    B, T, D = x.shape
    K = w1.shape[0]
    U = g.shape[1]
    assert (B, T, D, K, U) == (2, 1000, 512, 31, 8)
    NL = D // 128
    S1 = T // 2
    S2 = S1 // 2
    m1, m2 = 2 ** L1, 2 ** L2
    P1, P2 = 3 ** L1, 3 ** L2
    G1, G2 = 16 // m1, 16 // m2
    NB1 = -(-S1 // (m1 * 8)) * 8
    NB2 = -(-S2 // (m2 * 8)) * 8
    R1, R2 = B * NB1, B * NB2
    A1 = 2 * m1 * (NB1 + G1) + 16
    T1, T2 = _w_terms(L1), _w_terms(L2)
    assert m1 == 2 * m2
    HP = 8
    HR = HP + NB1 + 8
    X2R = NB2 + 8
    TC = 50
    NCH = S2 // TC

    groups = [(gg, ph) for gg in range(2) for ph in range(2)]

    def tap_index(ph, j):
        return 2 * j + ph

    def kernel(x_hbm, w1_hbm, w2_hbm, g_hbm, wf_hbm, wg_hbm, wo_hbm, o_hbm,
               x_v, w1_v, w2_v, g_v, wf_v, wg_v, wo_v,
               a1, xt1, y1, h_v, xt2, y2, f_v, fe_v, o_v,
               sem_x, sem_w1, sem_w2, sem_s, sem_o):

        def w_copy(hbm, v, sem, i):
            return pltpu.make_async_copy(hbm.at[i], v.at[i], sem.at[i])

        def grp_taps(q):
            gg, ph = groups[q]
            return [t for t in (tap_index(ph, 8 * gg + j) for j in range(8)) if t < K]

        def start_grp(hbm, v, sem, q):
            for t in grp_taps(q):
                w_copy(hbm, v, sem, t).start()

        small = [pltpu.make_async_copy(s, d, sem_s.at[i]) for i, (s, d) in
                 enumerate([(g_hbm, g_v), (wf_hbm, wf_v), (wg_hbm, wg_v), (wo_hbm, wo_v)])]

        xc = [pltpu.make_async_copy(x_hbm.at[b], x_v.at[b], sem_x.at[b]) for b in range(B)]
        for c in xc:
            c.start()
        start_grp(w1_hbm, w1_v, sem_w1, 0)

        for b in range(B):
            for lt in range(NL):
                a1[b, lt, 0:16, :] = jnp.zeros((16, 128), F32)
                a1[b, lt, 16 + T:A1, :] = jnp.zeros((A1 - 16 - T, 128), F32)
            for r in range(m1):
                h_v[r, b, 0:HP, :] = jnp.zeros((HP, D), F32)
                h_v[r, b, HP + NB1:HR, :] = jnp.zeros((HR - HP - NB1, D), F32)
        for b in range(B):
            xc[b].wait()
            for lt in range(NL):
                a1[b, lt, 16:16 + T, :] = x_v[b, :, 128 * lt:128 * lt + 128].astype(F32)

        def xform1(gg, ph):
            for b in range(B):
                for i in range(0, NB1, 16):
                  for lt in range(NL):
                    base = 2 * m1 * (i + gg) + ph + 1
                    xs = [a1[b, lt, pl.ds(base + 2 * c, 16, stride=2 * m1), :]
                          for c in range(2 * m1 - 1)]
                    vals = _x_tree(xs)
                    for p in range(P1):
                        xt1[gg, ph, p, b * NB1 + i:b * NB1 + i + 16,
                            128 * lt:128 * lt + 128] = vals[p].astype(BF16)

        def wsum(v, taps):
            taps = [t for t in taps if t < K]
            if not taps:
                return None
            if len(taps) == 1:
                return v[taps[0]]
            s = v[taps[0]].astype(F32)
            for t in taps[1:]:
                s = s + v[t].astype(F32)
            return s.astype(BF16)

        first = True
        for q, (gg, ph) in enumerate(groups):
            for t in grp_taps(q):
                w_copy(w1_hbm, w1_v, sem_w1, t).wait()
            if q + 1 < len(groups):
                start_grp(w1_hbm, w1_v, sem_w1, q + 1)
            else:
                for c in small:
                    c.start()
            start_grp(w2_hbm, w2_v, sem_w2, q)
            for sub in range(8 // m1):
                gi = gg * (8 // m1) + sub
                xform1(gi, ph)
                for p in range(P1):
                    w = wsum(w1_v, [tap_index(ph, m1 * gi + t) for t in T1[p]])
                    if w is None:
                        continue
                    d = jnp.dot(xt1[gi, ph, p], w, preferred_element_type=F32)
                    if first:
                        y1[p] = d
                    else:
                        y1[p] += d
                first = False

        for b in range(B):
            for i in range(0, NB1, 8):
                r0 = b * NB1 + i
                outs = _y_tree([y1[p, r0:r0 + 8, :] for p in range(P1)])
                for r in range(m1):
                    hv = _gelu(outs[r])
                    if m1 * (i + 7) + r >= S1:
                        kk = jax.lax.broadcasted_iota(jnp.int32, (8, D), 0) + i
                        hv = jnp.where(m1 * kk + r < S1, hv, 0.0)
                    h_v[r, b, HP + i:HP + i + 8, :] = hv.astype(BF16).astype(F32)

        for ph in range(2):
            for b in range(B):
                for i in range(0, X2R, 8):
                    xs = []
                    for c in range(2 * m2 - 1):
                        q = 2 * c + ph - 15 + 16
                        r, dk = q % m1, q // m1 - 16 // m1
                        st = HP + i + dk
                        if st + 8 <= HR:
                            xs.append(h_v[r, b, st:st + 8, :])
                        else:
                            xs.append(jnp.zeros((8, D), F32))
                    vals = _x_tree(xs)
                    for p in range(P2):
                        xt2[ph, p, b, i:i + 8, :] = vals[p]

        for t in range(K):
            w_copy(w2_hbm, w2_v, sem_w2, t).wait()
        for c in small:
            c.wait()
        for p in range(P2):
            acc = None
            for gi in range(G2):
                for ph in range(2):
                    w = wsum(w2_v, [tap_index(ph, m2 * gi + t) for t in T2[p]])
                    if w is None:
                        continue
                    lhs = jnp.concatenate(
                        [xt2[ph, p, b, gi:gi + NB2, :] for b in range(B)], axis=0).astype(BF16)
                    d = jnp.dot(lhs, w, preferred_element_type=F32)
                    acc = d if acc is None else acc + d
            y2[p] = acc

        for i in range(0, R2, 16):
            outs = _y_tree([y2[p, i:i + 16, :] for p in range(P2)])
            for r in range(m2):
                f_v[r * R2 + i:r * R2 + i + 16, :] = _gelu(outs[r]).astype(BF16)

        fe_v[...] = jnp.dot(f_v[...], wf_v[...], preferred_element_type=F32).astype(BF16).astype(F32)
        ge = jnp.dot(g_v[...].reshape(B * U, D), wg_v[...],
                     preferred_element_type=F32).astype(BF16).astype(F32)
        oc = []
        for b in range(B):
            geb = ge[b * U:(b + 1) * U]
            for ch in range(NCH):
                rows = []
                for t in range(ch * TC, (ch + 1) * TC):
                    row = (t % m2) * R2 + b * NB2 + t // m2
                    rows.append(jnp.tanh(fe_v[row:row + 1, :] + geb))
                j = jnp.concatenate(rows, axis=0).astype(BF16)
                o = jnp.dot(j, wo_v[...], preferred_element_type=F32).astype(BF16)
                o_v[b, ch * TC:(ch + 1) * TC] = o.reshape(TC, U, D)
                c = pltpu.make_async_copy(o_v.at[b, pl.ds(ch * TC, TC)],
                                          o_hbm.at[b, pl.ds(ch * TC, TC)],
                                          sem_o.at[b * NCH + ch])
                c.start()
                oc.append(c)
        for c in oc:
            c.wait()

    scratch = [
        pltpu.VMEM((B, T, D), BF16),
        pltpu.VMEM((K, D, D), BF16),
        pltpu.VMEM((K, D, D), BF16),
        pltpu.VMEM((B, U, D), BF16),
        pltpu.VMEM((D, D), BF16),
        pltpu.VMEM((D, D), BF16),
        pltpu.VMEM((D, D), BF16),
        pltpu.VMEM((B, NL, A1, 128), F32),
        pltpu.VMEM((G1, 2, P1, R1, D), BF16),
        pltpu.VMEM((P1, R1, D), F32),
        pltpu.VMEM((m1, B, HR, D), F32),
        pltpu.VMEM((2, P2, B, X2R, D), F32),
        pltpu.VMEM((P2, R2, D), F32),
        pltpu.VMEM((m2 * R2, D), BF16),
        pltpu.VMEM((m2 * R2, D), F32),
        pltpu.VMEM((B, S2, U, D), BF16),
        pltpu.SemaphoreType.DMA((B,)),
        pltpu.SemaphoreType.DMA((K,)),
        pltpu.SemaphoreType.DMA((K,)),
        pltpu.SemaphoreType.DMA((4,)),
        pltpu.SemaphoreType.DMA((B * NCH,)),
    ]
    any_spec = pl.BlockSpec(memory_space=pl.ANY)
    return pl.pallas_call(
        kernel,
        in_specs=[any_spec] * 7,
        out_specs=any_spec,
        out_shape=jax.ShapeDtypeStruct((B, S2, U, D), BF16),
        scratch_shapes=scratch,
        compiler_params=pltpu.CompilerParams(vmem_limit_bytes=112 * 2 ** 20),
    )(x, w1, w2, g, w_f, w_g, w_o)
```

```python
import numpy as np
import jax
import jax.numpy as jnp
import jax.experimental.pallas as pl
import jax.experimental.pallas.tpu as pltpu

PROFILE = False
F32 = jnp.float32
BF16 = jnp.bfloat16

L1 = 4
L2 = 3
LO1 = 2
LO2 = 2
KC = 128
NC = 128
YC = 128
XFIRST = 4
WSTART = 1
NFIRST = 0
NAHEAD = 8


def _w_terms(L):
    G = np.array([[1, 0], [1, 1], [0, 1]])
    M = np.eye(1, dtype=int)
    for _ in range(L):
        M = np.kron(G, M)
    return [[int(t) for t in np.nonzero(r)[0]] for r in M]


def _x_tree(xs):
    if len(xs) == 1:
        return list(xs)
    h = (len(xs) + 1) // 4
    n = 2 * h - 1
    x0, x1, x2 = xs[0:n], xs[h:h + n], xs[2 * h:2 * h + n]
    return (_x_tree([a - b for a, b in zip(x0, x1)]) + _x_tree(list(x1))
            + _x_tree([a - b for a, b in zip(x2, x1)]))


def _y_tree(ys):
    if len(ys) == 1:
        return list(ys)
    n = len(ys) // 3
    a, b, c = _y_tree(ys[:n]), _y_tree(ys[n:2 * n]), _y_tree(ys[2 * n:])
    return [u + v for u, v in zip(a, b)] + [u + v for u, v in zip(b, c)]


class _Scopes:
    def __init__(self):
        self.cur = None

    def mark(self, name):
        if not PROFILE:
            return
        if self.cur is not None:
            self.cur.__exit__(None, None, None)
        self.cur = jax.named_scope(name) if name else None
        if self.cur is not None:
            self.cur.__enter__()


def _gelu(x):
    c = float(np.sqrt(2.0 / np.pi))
    return 0.5 * x * (1.0 + jnp.tanh(c * (x + 0.044715 * (x * x * x))))


@jax.jit
def pallas_standalone__seq2seq_rnn_t_joint__speech_kernel(
    x: jax.Array,
    w1: jax.Array,
    w2: jax.Array,
    g: jax.Array,
    w_f: jax.Array,
    w_g: jax.Array,
    w_o: jax.Array,
):
    B, T, D = x.shape
    K = w1.shape[0]
    U = g.shape[1]
    assert (B, T, D, K, U) == (2, 1000, 512, 31, 8)
    NL = D // 128
    S1 = T // 2
    S2 = S1 // 2
    m1, m2 = 2 ** L1, 2 ** L2
    P1, P2 = 3 ** L1, 3 ** L2
    G1, G2 = 16 // m1, 16 // m2
    NB1 = -(-S1 // (m1 * 16)) * 16
    NB2 = -(-S2 // (m2 * 16)) * 16
    R1, R2 = B * NB1, B * NB2
    KB = (2 * m1 // 16) * (NB1 + G1) + 1
    PITCH = 17
    A1 = PITCH * KB
    assert m1 == 2 * m2
    HP = 8
    HR = HP + R1 + 8
    TC = 50
    NCH = S2 // TC

    def orders(L, LO):
        li = L - LO
        tr = _w_terms(li)
        io = sorted(range(3 ** li), key=lambda i: (max(tr[i]), -min(tr[i]) - 10 * (len(tr[i]) == 1)))
        seq = []
        for i in io:
            for o in range(2 ** LO):
                for t in tr[i]:
                    if o * 2 ** li + t not in seq:
                        seq.append(o * 2 ** li + t)
        return io, seq

    IO1, SEQ1 = orders(L1, LO1)
    IO2, SEQ2 = orders(L2, LO2)

    def tap1(q, pos):
        return 2 * (m1 * (q % G1) + SEQ1[pos]) + q // G1

    def tap2(q, pos):
        return 2 * (m2 * (q % G2) + SEQ2[pos]) + q // G2

    def kernel(x_hbm, w1_hbm, w2_hbm, g_hbm, wf_hbm, wg_hbm, wo_hbm, o_hbm,
               x_v, w1_v, w2_v, g_v, wf_v, wg_v, wo_v,
               a1, xt1, y1, h_v, xt2, y2, f_v, fe_v, o_v,
               sem_x, sem_w1, sem_w2, sem_s, sem_o):
        sc = _Scopes()
        sc.mark('prologue')

        def c1(t):
            return pltpu.make_async_copy(w1_hbm.at[t], w1_v.at[t], sem_w1.at[t])

        def c2(t):
            return pltpu.make_async_copy(w2_hbm.at[t], w2_v.at[t], sem_w2.at[t])

        small = [pltpu.make_async_copy(s, d, sem_s.at[i]) for i, (s, d) in
                 enumerate([(g_hbm, g_v), (wf_hbm, wf_v), (wg_hbm, wg_v), (wo_hbm, wo_v)])]

        stream = ([(c1, tap1(q, p_)) for q in range(2 * G1) for p_ in range(m1)]
                  + [(c2, tap2(q, p_)) for q in range(2 * G2) for p_ in range(m2)])

        def issue(n):
            if n < len(stream):
                f, t = stream[n]
                if t < K:
                    f(t).start()
            elif n == len(stream):
                for c in small:
                    c.start()

        def streamer(q, nq, m, base, cp, taps, seq):
            waited = set()

            def need(jjs):
                jjs = [jj for jj in jjs if jj not in waited]
                if not jjs:
                    return
                waited.update(jjs)
                for jj in jjs:
                    if jj != m - 1:
                        cp(taps[jj]).wait()
                for qq in range(nq):
                    def go(qq=qq):
                        if m - 1 in jjs and qq < nq - 1:
                            cp(2 * (m * (qq % (nq // 2)) + m - 1) + qq // (nq // 2)).wait()
                        for jj in jjs:
                            issue(base + m * qq + seq.index(jj) + NAHEAD)
                    pl.when(q == qq)(go)
            return need

        XS = [(0, 256), (256, 256), (512, 256), (768, T - 768)]
        xc = [pltpu.make_async_copy(x_hbm.at[:, pl.ds(a_, n_)], x_v.at[:, pl.ds(a_, n_)],
                                    sem_x.at[j]) for j, (a_, n_) in enumerate(XS)]
        for c in xc[:XFIRST]:
            c.start()
        for n in range(NFIRST):
            issue(n)

        w1_v[K] = jnp.zeros((D, D), BF16)
        w2_v[K] = jnp.zeros((D, D), BF16)
        y1[...] = jnp.zeros(y1.shape, F32)
        y2[...] = jnp.zeros(y2.shape, F32)
        for b in range(B):
            for lt in range(NL):
                a1[b, lt, 0:16, :] = jnp.zeros((16, 128), F32)
                for k in range(1 + T // 16, KB):
                    a1[b, lt, PITCH * k:PITCH * k + 16, :] = jnp.zeros((16, 128), F32)
        for r in range(m1):
            h_v[r, 0:HP, :] = jnp.zeros((HP, D), F32)
            h_v[r, HP + R1:HR, :] = jnp.zeros((HR - HP - R1, D), F32)
        for j, (a_, n_) in enumerate(XS):
            xc[j].wait()
            if j + XFIRST < len(XS):
                xc[j + XFIRST].start()
            if j == WSTART:
                for n in range(NFIRST, NAHEAD):
                    issue(n)
            for b in range(B):
                for k in range(a_ // 16, -(-(a_ + n_) // 16)):
                    n = min(16, T - 16 * k)
                    xv = x_v[b, 16 * k:16 * k + n, :].astype(F32)
                    for lt in range(NL):
                        a1[b, lt, PITCH * (k + 1):PITCH * (k + 1) + n, :] = (
                            xv[:, 128 * lt:128 * lt + 128])

        def pack(u, v):
            return pltpu.pack_elementwise([u, v], packed_dtype=BF16)

        def kara_group(v, taps, L, LO, io, xt, q, y, need):
            li = L - LO
            ni, mi = 3 ** li, 2 ** li
            trs = _w_terms(li)

            def tree(vals):
                if len(vals) == 1:
                    return vals
                h = len(vals) // 2
                a_, c_ = tree(vals[:h]), tree(vals[h:])
                return a_ + [(u[0] + w_[0], None) for u, w_ in zip(a_, c_)] + c_

            for i in io:
                tr = trs[i]
                tss = [[taps[o * mi + t] for t in tr] for o in range(2 ** LO)]
                need([o * mi + t for o in range(2 ** LO) for t in tr])
                for n0 in range(0, D, NC):
                    res = {}
                    for r in range(0, D, KC):
                        vals = []
                        for ts in tss:
                            s_ = None
                            for t in ts:
                                u = v[t, r:r + KC, n0:n0 + NC].astype(F32)
                                s_ = u if s_ is None else s_ + u
                            vals.append((s_, ts[0] if len(ts) == 1 else None))
                        for o, (val, rw) in enumerate(tree(vals)):
                            w = v[rw, r:r + KC, n0:n0 + NC] if rw is not None else val.astype(BF16)
                            lhs = pltpu.bitcast(xt[q, o * ni + i, :, r:r + KC], BF16)
                            d = jnp.dot(lhs, w, preferred_element_type=F32)
                            res[o] = d if o not in res else res[o] + d
                            if r + KC == D:
                                y[o * ni + i, :, n0:n0 + NC] += res.pop(o)

        gpb = 2 * m1 // 16
        for q in range(2 * G1):
            gi, ph = q % G1, q // G1
            for i in range(0, NB1, 8):
                for lt in range(NL):
                    vals = []
                    for b in range(B):
                        xs = []
                        for c in range(2 * m1 - 1):
                            qq = ph + 1 + 2 * c
                            base = PITCH * (gpb * (i + gi) + qq // 16) + qq % 16
                            xs.append(a1[b, lt, pl.ds(base, 8, stride=gpb * PITCH), :])
                        vals.append(_x_tree(xs))
                    for p in range(P1):
                        xt1[q, p, i:i + 8, 128 * lt:128 * lt + 128] = pack(vals[0][p], vals[1][p])
        sc.mark('c1')

        def c1_body(q, carry):
            taps = [2 * (m1 * (q % G1) + j) + q // G1 for j in range(m1)]
            kara_group(w1_v, taps, L1, LO1, IO1, xt1, q, y1,
                       streamer(q, 2 * G1, m1, 0, c1, taps, SEQ1))
            return carry

        jax.lax.fori_loop(0, 2 * G1, c1_body, 0)

        sc.mark('y1')
        for i in range(0, R1, 8):
            for lt in range(0, D, YC):
                outs = _y_tree([y1[p, i:i + 8, lt:lt + YC] for p in range(P1)])
                for r in range(m1):
                    hv = _gelu(outs[r])
                    if m1 * ((i + 7) // 2) + r >= S1:
                        kk = (jax.lax.broadcasted_iota(jnp.int32, (8, YC), 0) + i) >> 1
                        hv = jnp.where(m1 * kk + r < S1, hv, 0.0)
                    h_v[r, HP + i:HP + i + 8, lt:lt + YC] = hv.astype(BF16).astype(F32)

        sc.mark('x2')
        for q in range(2 * G2):
            gi, ph = q % G2, q // G2
            for i in range(0, R2 // 2, 8):
                for lt in range(0, D, 128):
                    vals = []
                    for e in range(2):
                        xs = []
                        for c in range(2 * m2 - 1):
                            qq = 2 * c + ph + 1
                            st = HP + e * (R2 // 2) + i + B * (gi + qq // m1 - 16 // m1)
                            xs.append(h_v[qq % m1, st:st + 8, lt:lt + 128])
                        vals.append(_x_tree(xs))
                    for p in range(P2):
                        xt2[q, p, i:i + 8, lt:lt + 128] = pack(vals[0][p], vals[1][p])
        sc.mark('c2')

        def c2_body(q, carry):
            taps = [2 * (m2 * (q % G2) + j) + q // G2 for j in range(m2)]
            kara_group(w2_v, taps, L2, LO2, IO2, xt2, q, y2,
                       streamer(q, 2 * G2, m2, 32, c2, taps, SEQ2))
            return carry

        jax.lax.fori_loop(0, 2 * G2, c2_body, 0)
        for c in small:
            c.wait()
        sc.mark('y2')

        for i in range(0, R2, 16):
            outs = _y_tree([y2[p, i:i + 16, :] for p in range(P2)])
            for r in range(m2):
                f_v[r * R2 + i:r * R2 + i + 16, :] = _gelu(outs[r]).astype(BF16)

        sc.mark('joint')
        fe_v[...] = jnp.dot(f_v[...], wf_v[...], preferred_element_type=F32).astype(BF16).astype(F32)
        ge = jnp.dot(g_v[...].reshape(B * U, D), wg_v[...],
                     preferred_element_type=F32).astype(BF16).astype(F32)
        oc = []
        for b in range(B):
            geb = ge[b * U:(b + 1) * U]
            for ch in range(NCH):
                rows = []
                for t in range(ch * TC, (ch + 1) * TC):
                    nat = 2 * (t // m2) + b
                    row = (t % m2) * R2 + 2 * (nat % (R2 // 2)) + nat // (R2 // 2)
                    rows.append(jnp.tanh(fe_v[row:row + 1, :] + geb))
                j = jnp.concatenate(rows, axis=0).astype(BF16)
                o = jnp.dot(j, wo_v[...], preferred_element_type=F32).astype(BF16)
                o_v[b, ch * TC:(ch + 1) * TC] = o.reshape(TC, U, D)
                c = pltpu.make_async_copy(o_v.at[b, pl.ds(ch * TC, TC)],
                                          o_hbm.at[b, pl.ds(ch * TC, TC)],
                                          sem_o.at[b * NCH + ch])
                c.start()
                oc.append(c)
        sc.mark('tail')
        for c in oc:
            c.wait()
        sc.mark(None)

    scratch = [
        pltpu.VMEM((B, T, D), BF16),
        pltpu.VMEM((K + 1, D, D), BF16),
        pltpu.VMEM((K + 1, D, D), BF16),
        pltpu.VMEM((B, U, D), BF16),
        pltpu.VMEM((D, D), BF16),
        pltpu.VMEM((D, D), BF16),
        pltpu.VMEM((D, D), BF16),
        pltpu.VMEM((B, NL, A1, 128), F32),
        pltpu.VMEM((2 * G1, P1, R1 // 2, D), jnp.uint32),
        pltpu.VMEM((P1, R1, D), F32),
        pltpu.VMEM((m1, HR, D), F32),
        pltpu.VMEM((2 * G2, P2, R2 // 2, D), jnp.uint32),
        pltpu.VMEM((P2, R2, D), F32),
        pltpu.VMEM((m2 * R2, D), BF16),
        pltpu.VMEM((m2 * R2, D), F32),
        pltpu.VMEM((B, S2, U, D), BF16),
        pltpu.SemaphoreType.DMA((4,)),
        pltpu.SemaphoreType.DMA((K + 1,)),
        pltpu.SemaphoreType.DMA((K + 1,)),
        pltpu.SemaphoreType.DMA((4,)),
        pltpu.SemaphoreType.DMA((B * NCH,)),
    ]
    any_spec = pl.BlockSpec(memory_space=pl.ANY)
    return pl.pallas_call(
        kernel,
        grid=(1,),
        in_specs=[any_spec] * 7,
        out_specs=any_spec,
        out_shape=jax.ShapeDtypeStruct((B, S2, U, D), BF16),
        scratch_shapes=scratch,
        compiler_params=pltpu.CompilerParams(vmem_limit_bytes=112 * 2 ** 20),
    )(x, w1, w2, g, w_f, w_g, w_o)
```
